```python
import os as _os
_os.environ.setdefault("JAX_PLATFORMS", "cpu")
import jax
import jax.numpy as jnp

def _softmax(x, axis=-1):
    return jax.nn.softmax(x, axis=axis)
def _gelu(x):
    return jax.nn.gelu(x, approximate=True)
def _silu(x):
    return jax.nn.silu(x)
def _sigmoid(x):
    return jax.nn.sigmoid(x)
def _layernorm(x, axis=-1, eps=1e-5):
    m = jnp.mean(x, axis=axis, keepdims=True)
    v = jnp.var(x, axis=axis, keepdims=True)
    return (x - m) / jnp.sqrt(v + eps)
def _scatter_add(tgt, idx, src, axis=0):
    return tgt.at[idx].add(src)
def _segment_sum(src, seg, n):
    return jax.ops.segment_sum(src, seg, n)
class _Rng:
    def __init__(self, key):
        self._k = key
    def _next(self):
        self._k, sub = jax.random.split(self._k)
        return sub
    def normal(self, shape):
        return jax.random.normal(self._next(), shape, dtype=jnp.bfloat16)
    def randint(self, lo, hi, shape):
        return jax.random.randint(self._next(), shape, lo, hi, dtype=jnp.int32)
    def uniform(self, shape, lo=0.0, hi=1.0):
        return jax.random.uniform(self._next(), shape, jnp.bfloat16, lo, hi)
    def permutation(self, n):
        return jax.random.permutation(self._next(), n)


kernel_name = 'gated_mix__mha_block__softmax_full_mha__prompt'

def setup_inputs():
    _rng = _Rng(jax.random.key(int.from_bytes(__import__("os").urandom(4), "little")))
    _w = (lambda a: (lambda t: t.astype(jnp.bfloat16) if jnp.issubdtype(t.dtype, jnp.floating) else t)(jnp.asarray(a)))
    def _A_setup():
        B, S, D, H = 1, 2048, 448, 16
        return {
            "x": _w((lambda *s: _rng.normal(s) * 0.05)(B, S, D)),
            "wqkv": _w((lambda *s: _rng.normal(s) * 0.4)(D, 3 * D)),
            "wo": _w((lambda *s: _rng.normal(s) * 0.05)(D, D)),
        }
    _A_in = _A_setup()

    def _B_setup():
        B, S, D = 1, 2048, 448
        return {
            "x": _w((lambda *s: _rng.normal(s) * 0.05)(B, S, D)),
            "wqkv": _w((lambda *s: _rng.normal(s) * 0.4)(D, 3 * D)),
            "wo": _w((lambda *s: _rng.normal(s) * 0.05)(D, D)),
        }
    _B_in = _B_setup()

    return {
        "A_x": _A_in["x"],
        "A_wqkv": _A_in["wqkv"],
        "A_wo": _A_in["wo"],
        "B_x": _B_in["x"],
        "B_wqkv": _B_in["wqkv"],
        "B_wo": _B_in["wo"],
        "gate_w": _w((lambda *s: _rng.normal(s) * 0.05)(448) * 16.0),
    }

def reference(A_x, A_wqkv, A_wo, B_x, B_wqkv, B_wo, gate_w):
    def _A_ref(x, wqkv, wo):
        B, S, D = x.shape
        H = 16
        Dh = D // H
        qkv = (lambda x, *d: x.transpose(*d))((x @ wqkv).reshape(B, S, 3, H, Dh), 2, 0, 3, 1, 4)
        q, k, v = qkv[0], qkv[1], qkv[2]
        scores = jnp.einsum("bhqd,bhkd->bhqk", q, k) * (Dh ** -0.5)
        p = _softmax(scores, axis=-1)
        o = jnp.einsum("bhqk,bhkd->bhqd", p, v)
        return (lambda x, *d: x.transpose(*d))(o, 0, 2, 1, 3).reshape(B, S, D) @ wo

    def _B_ref(x, wqkv, wo):
        B, S, D = x.shape
        H = 16; Dh = D // H
        qkv = (lambda x, *d: x.transpose(*d))((x @ wqkv).reshape(B, S, 3, H, Dh), 2, 0, 3, 1, 4)
        q, k, v = qkv[0], qkv[1], qkv[2]
        scale = Dh ** -0.5
        scores = jnp.einsum("bhqd,bhkd->bhqk", q, k) * scale
        p = _softmax(scores, axis=-1)
        o = jnp.einsum("bhqk,bhkd->bhqd", p, v)
        return (lambda x, *d: x.transpose(*d))(o, 0, 2, 1, 3).reshape(B, S, D) @ wo

    x = A_x
    g = _sigmoid((x * gate_w).sum(-1, keepdims=True))
    a = _A_ref(x, A_wqkv, A_wo)
    b = _B_ref(x, B_wqkv, B_wo)
    return g * a + (1 - g) * b
```

```python
import functools
import jax, jax.numpy as jnp, numpy as np
from jax.experimental import pallas as pl
from jax.experimental.pallas import tpu as pltpu

S, D, H, DH = 2048, 448, 16, 28
HP = 32
NSLAB = 4
LOG2E = 1.4426950408889634
F32, BF16 = jnp.float32, jnp.bfloat16

def nt(a, b):
    return jax.lax.dot_general(a, b, (((1,), (1,)), ((), ())), preferred_element_type=F32)
def nn(a, b):
    return jnp.dot(a, b, preferred_element_type=F32)

def make(TQ=512, KB1=128, KB2=128, U=3, TRIP=None, PROJ_LOOP=True, STOP=None):
    NC = S // TQ
    NITEM = 32 * NC
    def kern(xT_hbm, wA_hbm, woA_hbm, wB_hbm, woB_hbm, gate_hbm, outT_hbm,
             xT_s, w_s, wo_s, gate_s, out_s, x_s, wk_s, wqT_s, wvT_s, woT_s,
             k_s, q_s, vT_s, oT_s, s0, s1, g_s, sems):
        cps = [pltpu.make_async_copy(xT_hbm.at[0], xT_s, sems.at[0]),
               pltpu.make_async_copy(wA_hbm, w_s.at[0], sems.at[1]),
               pltpu.make_async_copy(gate_hbm, gate_s, sems.at[2]),
               pltpu.make_async_copy(woA_hbm, wo_s.at[0], sems.at[3]),
               pltpu.make_async_copy(wB_hbm, w_s.at[1], sems.at[4]),
               pltpu.make_async_copy(woB_hbm, wo_s.at[1], sems.at[5])]
        cps[1].start(); cps[0].start(); cps[2].start()

        starts = [0, 0, 128, 256]
        def sel(j):
            wdt = min(256, D - starts[j])
            r = jax.lax.broadcasted_iota(jnp.int32, (128, wdt), 0)
            c = jax.lax.broadcasted_iota(jnp.int32, (128, wdt), 1)
            rr = r & (HP - 1)
            src = 112 * j - starts[j] + DH * (r >> 5) + rr
            return jnp.where((c == src) & (rr < DH), 1.0, 0.0).astype(BF16)
        sels = [sel(j) for j in range(NSLAB)]

        def prep_qkv(b):
            wq = w_s[b, :, 0:512].astype(F32)
            wqT = (wq.T * (DH ** -0.5 * LOG2E)).astype(BF16)
            for j in range(NSLAB):
                t = b * NSLAB + j
                wqT_s[t] = wqT[112 * j:112 * j + 112, :]
                o = D + 112 * j
                wk_s[t] = w_s[b, :, o:o + 128]
                wdt = sels[j].shape[1]
                o = 2 * D + starts[j]
                wvT_s[t] = nt(sels[j], w_s[b, :, o:o + wdt]).astype(BF16)
        def prep_wo(b):
            woT = wo_s[b].astype(F32).T.astype(BF16)
            for j in range(NSLAB):
                wdt = sels[j].shape[1]
                woT_s[b * NSLAB + j] = nt(woT[:, starts[j]:starts[j] + wdt], sels[j]).astype(BF16)

        rows = jax.lax.broadcasted_iota(jnp.int32, (128, S), 0)
        def proj(t):
            k_s[t] = nn(x_s[...], wk_s[t]).astype(BF16)
            q_s[t, 0:112, :] = nn(wqT_s[t], xT_s[...]).astype(BF16)
            q_s[t, 112:128, :] = jnp.zeros((16, S), BF16)
            vT_s[t] = jnp.where((rows & (HP - 1)) == DH, 1.0, nn(wvT_s[t], xT_s[...])).astype(BF16)

        cps[1].wait()
        prep_qkv(0)
        cps[0].wait()
        cps[4].start(); cps[3].start(); cps[5].start()
        cps[2].wait()
        g8 = jnp.broadcast_to(gate_s[...].reshape(1, D), (16, D))
        g = jax.nn.sigmoid(nn(g8, xT_s[...])[0:1, :])
        g_s[0] = jnp.broadcast_to(g, (8, S))
        g_s[1] = jnp.broadcast_to(1.0 - g, (8, S))
        x_s[...] = xT_s[...].astype(F32).T.astype(BF16)
        if PROJ_LOOP:
            jax.lax.fori_loop(0, 4, lambda t, _: (proj(t), 0)[1], 0)
        else:
            for t in range(4): proj(t)
        cps[4].wait(); cps[3].wait(); cps[5].wait()
        prep_qkv(1); prep_wo(0); prep_wo(1)
        if PROJ_LOOP:
            jax.lax.fori_loop(4, 8, lambda t, _: (proj(t), 0)[1], 0)
        else:
            for t in range(4, 8): proj(t)

        def get_q(n):
            hh = n // NC; c = n % NC
            t = hh // 4; i = hh % 4
            c0 = pl.multiple_of(c * TQ, TQ)
            q = q_s[t, :, pl.ds(c0, TQ)]
            ll = jax.lax.broadcasted_iota(jnp.int32, (128, TQ), 0)
            return jnp.where((ll >= i * DH) & (ll < i * DH + DH), q, jnp.zeros_like(q)), t

        def pair(n1, sw, n2, sr, m2):
            do1 = n1 is not None; do2 = n2 is not None
            if do1:
                q, t1 = get_q(n1)
                m8 = jnp.full((8, TQ), -jnp.inf, F32)
            if do2:
                hh = n2 // NC; c = n2 % NC; t2 = hh // 4; i2 = hh % 4; b2 = hh // 16
                r0 = pl.multiple_of(i2 * HP, HP); c0 = pl.multiple_of(c * TQ, TQ)
                o = jnp.zeros((HP, TQ), F32)
            nb = S // max(KB1, KB2) if (do1 and do2) else 1
            for blk in range(nb):
                if do1:
                    for k0 in range(blk * S // nb, (blk + 1) * S // nb, KB1):
                        s = nn(k_s[t1, k0:k0 + KB1, :], q)
                        sw[k0:k0 + KB1, :] = s
                        m8 = jnp.maximum(m8, jnp.max(s.reshape(KB1 // 8, 8, TQ), axis=0))
                if do2:
                    for k0 in range(blk * S // nb, (blk + 1) * S // nb, KB2):
                        s = sr[k0:k0 + KB2, :].reshape(KB2 // 8, 8, TQ)
                        p = jnp.exp2(s - m2[None]).reshape(KB2, TQ).astype(BF16)
                        o = o + nn(vT_s[t2, pl.ds(r0, HP), k0:k0 + KB2], p)
            if do2:
                sc = g_s[b2, 0:1, pl.ds(c0, TQ)] / o[DH:DH + 1, :]
                oT_s[t2, pl.ds(r0, HP), pl.ds(c0, TQ)] = (o * sc).astype(BF16)
            if do1:
                return jnp.broadcast_to(jnp.max(m8, axis=0, keepdims=True), (8, TQ))
            return None

        if STOP != "proj":
            m0 = pair(0, s0, None, None, None)
            nbody = (NITEM - 2) // (2 * U)
            def body(t, m0):
                for u in range(U):
                    n = 2 * (t * U + u)
                    m1 = pair(n + 1, s1, n, s0, m0)
                    m0 = pair(n + 2, s0, n + 1, s1, m1)
                return m0
            m0 = jax.lax.fori_loop(0, TRIP if TRIP else nbody, body, m0)
            for n in range(2 * U * nbody, NITEM - 2, 2):
                m1 = pair(n + 1, s1, n, s0, m0)
                m0 = pair(n + 2, s0, n + 1, s1, m1)
            m1 = pair(NITEM - 1, s1, NITEM - 2, s0, m0)
            pair(None, None, NITEM - 1, s1, m1)
        else:
            oT_s[...] = vT_s[...]

        OC = 512
        def outp(c, _):
            c0 = pl.multiple_of(c * OC, OC)
            acc = nn(woT_s[0], oT_s[0, :, pl.ds(c0, OC)])
            for t in range(1, 8):
                acc = acc + nn(woT_s[t], oT_s[t, :, pl.ds(c0, OC)])
            out_s[:, pl.ds(c0, OC)] = acc.astype(BF16)
            pltpu.make_async_copy(out_s.at[:, pl.ds(c0, OC)], outT_hbm.at[0, :, pl.ds(c0, OC)], sems.at[6]).start()
            return 0
        jax.lax.fori_loop(0, S // OC, outp, 0)
        pltpu.make_async_copy(out_s, outT_hbm.at[0], sems.at[6]).wait()

    @jax.jit
    def f(A_x, A_wqkv, A_wo, B_x, B_wqkv, B_wo, gate_w):
        anyspec = pl.BlockSpec(memory_space=pl.ANY)
        outT = pl.pallas_call(
            kern,
            in_specs=[anyspec] * 6, out_specs=anyspec,
            out_shape=jax.ShapeDtypeStruct((1, D, S), BF16),
            scratch_shapes=[
                pltpu.VMEM((D, S), BF16), pltpu.VMEM((2, D, 3 * D), BF16), pltpu.VMEM((2, D, D), BF16),
                pltpu.VMEM((D,), BF16), pltpu.VMEM((D, S), BF16),
                pltpu.VMEM((S, D), BF16),
                pltpu.VMEM((8, D, 128), BF16), pltpu.VMEM((8, 112, D), BF16), pltpu.VMEM((8, 128, D), BF16),
                pltpu.VMEM((8, D, 128), BF16),
                pltpu.VMEM((8, S, 128), BF16),
                pltpu.VMEM((8, 128, S), BF16),
                pltpu.VMEM((8, 128, S), BF16), pltpu.VMEM((8, 128, S), BF16),
                pltpu.VMEM((S, TQ), F32), pltpu.VMEM((S, TQ), F32), pltpu.VMEM((2, 8, S), F32),
                pltpu.SemaphoreType.DMA((7,)),
            ],
            compiler_params=pltpu.CompilerParams(vmem_limit_bytes=110 * 2**20),
        )(jnp.swapaxes(A_x, 1, 2), A_wqkv, A_wo, B_wqkv, B_wo, gate_w)
        return jnp.swapaxes(outT, 1, 2)
    return f


_kernel = make(U=3)


@jax.jit
def pallas_gated_mix__mha_block__softmax_full_mha__prompt_kernel(
    A_x: jax.Array,
    A_wqkv: jax.Array,
    A_wo: jax.Array,
    B_x: jax.Array,
    B_wqkv: jax.Array,
    B_wo: jax.Array,
    gate_w: jax.Array,
):
    return _kernel(A_x, A_wqkv, A_wo, B_x, B_wqkv, B_wo, gate_w)
```

```python
import jax
import jax.numpy as jnp
from jax.experimental import pallas as pl
from jax.experimental.pallas import tpu as pltpu

S, D, H, DH = 2048, 448, 16, 28
HP = 32
NSLAB = 4
SW = 4 * DH
LOG2E = 1.4426950408889634
F32, BF16 = jnp.float32, jnp.bfloat16

TQ = 512
KB = 128
SKEW = 2
U = 7
XC = 4
OC = 512
NC = S // TQ
NITEM = 2 * H * NC
XW = S // XC


def _nn(a, b):
    return jnp.dot(a, b, preferred_element_type=F32)


def _kernel(xT_hbm, wA_hbm, woA_hbm, wB_hbm, woB_hbm, gate_hbm, outT_hbm,
            xT_s, w_s, wo_s, gate_s, out_s, wT_s, woT_s,
            k_s, q_s, vT_s, oT_s, s0, s1, g_s, sems, xsems):
    def xcp(c):
        c0 = pl.multiple_of(c * XW, XW)
        return pltpu.make_async_copy(
            xT_hbm.at[0, :, pl.ds(c0, XW)], xT_s.at[:, pl.ds(c0, XW)], xsems.at[c])

    cp_wA = pltpu.make_async_copy(wA_hbm, w_s.at[0], sems.at[0])
    cp_gate = pltpu.make_async_copy(gate_hbm, gate_s, sems.at[1])
    cp_wB = pltpu.make_async_copy(wB_hbm, w_s.at[1], sems.at[2])
    cp_woA = pltpu.make_async_copy(woA_hbm, wo_s.at[0:D, :], sems.at[3])
    cp_woB = pltpu.make_async_copy(woB_hbm, wo_s.at[D:2 * D, :], sems.at[4])
    out_sem = sems.at[5]

    def prep_qkv(b):
        wqT = (w_s[b, :, 0:512].astype(F32).T * (DH ** -0.5 * LOG2E)).astype(BF16)
        wkT = w_s[b, :, 384:896].astype(F32).T.astype(BF16)
        wvT = w_s[b, :, 2 * D:3 * D].astype(F32).T.astype(BF16)
        for j in range(NSLAB):
            t = b * NSLAB + j
            wT_s[t, 0:SW, :] = wqT[SW * j:SW * (j + 1), :]
            wT_s[t, SW:2 * SW, :] = wkT[64 + SW * j:64 + SW * (j + 1), :]
            wT_s[t, 2 * SW:3 * SW, :] = wvT[SW * j:SW * (j + 1), :]

    def proj(t, c0, W):
        r = _nn(wT_s[t], xT_s[:, pl.ds(c0, W)])
        zpad = jnp.zeros((128 - SW, W), F32)
        rows = jax.lax.broadcasted_iota(jnp.int32, (128, W), 0)
        qq = jnp.concatenate([r[0:SW], zpad], axis=0).astype(BF16)
        for i in range(4):
            q_s[4 * t + i, :, pl.ds(c0, W)] = jnp.where(
                (rows >= i * DH) & (rows < (i + 1) * DH), qq, jnp.zeros_like(qq))
        kk = jnp.concatenate([r[SW:2 * SW], zpad], axis=0)
        k_s[t, pl.ds(c0, W), :] = kk.T.astype(BF16)
        aux = jnp.where(jax.lax.broadcasted_iota(jnp.int32, (HP - DH, W), 0) == 0, 1.0, 0.0)
        parts = []
        for i in range(4):
            parts += [r[2 * SW + DH * i:2 * SW + DH * (i + 1)], aux]
        vT_s[t, :, pl.ds(c0, W)] = jnp.concatenate(parts, axis=0).astype(BF16)

    cp_wA.start()
    xcp(0).start()
    cp_gate.start()
    cp_wA.wait()
    for c in range(1, XC):
        xcp(c).start()
    prep_qkv(0)
    cp_gate.wait()
    g8 = jnp.broadcast_to(gate_s[...].reshape(1, D), (16, D))

    def chunk_a(c):
        xcp(c).wait()
        c0 = pl.multiple_of(c * XW, XW)
        g = jax.nn.sigmoid(_nn(g8, xT_s[:, pl.ds(c0, XW)])[0:1, :])
        g_s[0, :, pl.ds(c0, XW)] = jnp.broadcast_to(g, (8, XW))
        g_s[1, :, pl.ds(c0, XW)] = jnp.broadcast_to(1.0 - g, (8, XW))
        for t in range(NSLAB):
            proj(t, c0, XW)

    def loop_a(c, carry):
        @pl.when(c == 0)
        def _():
            cp_wB.start()
            cp_woA.start()
            cp_woB.start()
        chunk_a(c)
        return carry

    jax.lax.fori_loop(0, XC - 1, loop_a, 0)
    cp_wB.wait()
    cp_woA.wait()
    cp_woB.wait()
    chunk_a(XC - 1)
    prep_qkv(1)
    woT_s[...] = wo_s[...].astype(F32).T.astype(BF16)

    def loop_b(t, carry):
        proj(t, 0, S)
        return carry

    jax.lax.fori_loop(NSLAB, 2 * NSLAB, loop_b, 0)

    def pair(n1, sw, n2, sr, m2):
        do1 = n1 is not None
        do2 = n2 is not None
        if do1:
            h1 = n1 // NC
            t1 = h1 // 4
            q = q_s[h1, :, pl.ds(pl.multiple_of((n1 % NC) * TQ, TQ), TQ)]
            m8 = jnp.full((8, TQ), -jnp.inf, F32)
        if do2:
            h2 = n2 // NC
            t2 = h2 // 4
            r0 = pl.multiple_of((h2 % 4) * HP, HP)
            c0 = pl.multiple_of((n2 % NC) * TQ, TQ)
            o = jnp.zeros((HP, TQ), F32)

        a = list(range(0, S, KB)) if do1 else []
        bb = list(range(0, S, KB)) if do2 else []
        ia = ib = 0
        while ia < len(a) or ib < len(bb):
            if ia < len(a) and (ib >= len(bb) or a[ia] <= bb[ib] + SKEW * KB):
                k0 = a[ia]
                ia += 1
                s = _nn(k_s[t1, k0:k0 + KB, :], q)
                sw[k0:k0 + KB, :] = s
                m8 = jnp.maximum(m8, jnp.max(s.reshape(KB // 8, 8, TQ), axis=0))
            else:
                k0 = bb[ib]
                ib += 1
                s = sr[k0:k0 + KB, :].reshape(KB // 8, 8, TQ)
                p = jnp.exp2(s - m2[None]).reshape(KB, TQ).astype(BF16)
                o = o + _nn(vT_s[t2, pl.ds(r0, HP), k0:k0 + KB], p)
        if do2:
            sc = g_s[h2 // H, 0:1, pl.ds(c0, TQ)] / o[DH:DH + 1, :]
            oT_s[t2, pl.ds(r0, HP), pl.ds(c0, TQ)] = o * sc
        if do1:
            return jnp.broadcast_to(jnp.max(m8, axis=0, keepdims=True), (8, TQ))
        return None

    def outp(c, carry):
        c0 = pl.multiple_of(c * OC, OC)
        parts = []
        for t in range(2 * NSLAB):
            ot = oT_s[t, :, pl.ds(c0, OC)]
            parts += [ot[HP * i:HP * i + DH] for i in range(4)]
        acc = _nn(woT_s[...], jnp.concatenate(parts, axis=0).astype(BF16))
        out_s[:, pl.ds(c0, OC)] = acc.astype(BF16)
        pltpu.make_async_copy(
            out_s.at[:, pl.ds(c0, OC)], outT_hbm.at[0, :, pl.ds(c0, OC)], out_sem).start()
        return carry

    m0 = pair(0, s0, None, None, None)
    nbody = (NITEM - 2) // (2 * U)

    def body(it, m0):
        for u in range(U):
            n = 2 * (it * U + u)
            m1 = pair(n + 1, s1, n, s0, m0)
            m0 = pair(n + 2, s0, n + 1, s1, m1)
        return m0

    m0 = jax.lax.fori_loop(0, nbody, body, m0)
    for n in range(2 * U * nbody, NITEM - 2, 2):
        m1 = pair(n + 1, s1, n, s0, m0)
        m0 = pair(n + 2, s0, n + 1, s1, m1)
    m1 = pair(NITEM - 1, s1, NITEM - 2, s0, m0)
    pair(None, None, NITEM - 1, s1, m1)

    outp(0, 0)
    jax.lax.fori_loop(1, S // OC, outp, 0)
    pltpu.make_async_copy(out_s, outT_hbm.at[0], out_sem).wait()


@jax.jit
def pallas_gated_mix__mha_block__softmax_full_mha__prompt_kernel(
    A_x: jax.Array,
    A_wqkv: jax.Array,
    A_wo: jax.Array,
    B_x: jax.Array,
    B_wqkv: jax.Array,
    B_wo: jax.Array,
    gate_w: jax.Array,
):
    del B_x
    anyspec = pl.BlockSpec(memory_space=pl.ANY)
    outT = pl.pallas_call(
        _kernel,
        in_specs=[anyspec] * 6,
        out_specs=anyspec,
        out_shape=jax.ShapeDtypeStruct((1, D, S), BF16),
        scratch_shapes=[
            pltpu.VMEM((D, S), BF16),
            pltpu.VMEM((2, D, 3 * D), BF16),
            pltpu.VMEM((2 * D, D), BF16),
            pltpu.VMEM((D,), BF16),
            pltpu.VMEM((D, S), BF16),
            pltpu.VMEM((2 * NSLAB, 3 * SW, D), BF16),
            pltpu.VMEM((D, 2 * D), BF16),
            pltpu.VMEM((2 * NSLAB, S, 128), BF16),
            pltpu.VMEM((2 * H, 128, S), BF16),
            pltpu.VMEM((2 * NSLAB, 128, S), BF16),
            pltpu.VMEM((2 * NSLAB, 128, S), F32),
            pltpu.VMEM((S, TQ), F32),
            pltpu.VMEM((S, TQ), F32),
            pltpu.VMEM((2, 8, S), F32),
            pltpu.SemaphoreType.DMA((6,)),
            pltpu.SemaphoreType.DMA((XC,)),
        ],
        compiler_params=pltpu.CompilerParams(vmem_limit_bytes=110 * 2**20),
    )(jnp.swapaxes(A_x, 1, 2), A_wqkv, A_wo, B_wqkv, B_wo, gate_w)
    return jnp.swapaxes(outT, 1, 2)
```

```python
import jax
import jax.numpy as jnp
from jax.experimental import pallas as pl
from jax.experimental.pallas import tpu as pltpu

S, D, H, DH = 2048, 448, 16, 28
HP = 32
NSLAB = 4
SW = 4 * DH
LOG2E = 1.4426950408889634
F32, BF16 = jnp.float32, jnp.bfloat16

TQ = 512
KB = 128
SKEW = 2
U = 7
XC = 4
OC = 512
NC = S // TQ
NITEM = 2 * H * NC
XW = S // XC


def _nn(a, b):
    return jnp.dot(a, b, preferred_element_type=F32)


def _kernel(xT_hbm, wA_hbm, woA_hbm, wB_hbm, woB_hbm, gate_hbm, outT_hbm,
            xT_s, w_s, wo_s, gate_s, out_s, wT_s, woT_s,
            k_s, q_s, vT_s, oT_s, s0, s1, g_s, sems, xsems):
    def xcp(c):
        c0 = pl.multiple_of(c * XW, XW)
        return pltpu.make_async_copy(
            xT_hbm.at[0, :, pl.ds(c0, XW)], xT_s.at[:, pl.ds(c0, XW)], xsems.at[c])

    cp_w = [pltpu.make_async_copy(wA_hbm.at[:, a:b], w_s.at[0, :, a:b], sems.at[i])
            for i, (a, b) in ((0, (0, 512)), (6, (512, 896)), (7, (896, 3 * D)))]
    cp_gate = pltpu.make_async_copy(gate_hbm, gate_s, sems.at[1])
    cp_wB = pltpu.make_async_copy(wB_hbm, w_s.at[1], sems.at[2])
    cp_woA = pltpu.make_async_copy(woA_hbm, wo_s.at[0:D, :], sems.at[3])
    cp_woB = pltpu.make_async_copy(woB_hbm, wo_s.at[D:2 * D, :], sems.at[4])
    out_sem = sems.at[5]

    def prep_qkv(b, waits=None):
        wait = (lambda i: waits[i].wait()) if waits else (lambda i: None)
        wait(0)
        wqT = w_s[b, :, 0:512].astype(F32).T.astype(BF16)
        wait(1)
        wkT = w_s[b, :, 384:896].astype(F32).T.astype(BF16)
        wait(2)
        if waits:
            for c in range(1, XC):
                xcp(c).start()
        wvT = w_s[b, :, 2 * D:3 * D].astype(F32).T.astype(BF16)
        for j in range(NSLAB):
            t = b * NSLAB + j
            wT_s[t, SW:2 * SW, :] = wqT[SW * j:SW * (j + 1), :]
            wT_s[t, 0:SW, :] = wkT[64 + SW * j:64 + SW * (j + 1), :]
            wT_s[t, 2 * SW:3 * SW, :] = wvT[SW * j:SW * (j + 1), :]

    def proj(t, c0, W):
        r = _nn(wT_s[t], xT_s[:, pl.ds(c0, W)])
        zpad = jnp.zeros((128 - SW, W), F32)
        rows = jax.lax.broadcasted_iota(jnp.int32, (128, W), 0)
        qq = jnp.concatenate([r[SW:2 * SW] * (DH ** -0.5 * LOG2E), zpad], axis=0).astype(BF16)
        for i in range(4):
            q_s[4 * t + i, :, pl.ds(c0, W)] = jnp.where(
                (rows >= i * DH) & (rows < (i + 1) * DH), qq, jnp.zeros_like(qq))
        kk = jnp.concatenate([r[0:SW], zpad], axis=0)
        k_s[t, pl.ds(c0, W), :] = kk.T.astype(BF16)
        aux = jnp.where(jax.lax.broadcasted_iota(jnp.int32, (HP - DH, W), 0) == 0, 1.0, 0.0)
        parts = []
        for i in range(4):
            parts += [r[2 * SW + DH * i:2 * SW + DH * (i + 1)], aux]
        vT_s[t, :, pl.ds(c0, W)] = jnp.concatenate(parts, axis=0).astype(BF16)

    cp_w[0].start()
    xcp(0).start()
    cp_w[1].start()
    cp_w[2].start()
    cp_gate.start()
    prep_qkv(0, cp_w)
    cp_gate.wait()
    g8 = jnp.broadcast_to(gate_s[...].reshape(1, D), (16, D))

    def chunk_a(c):
        xcp(c).wait()
        c0 = pl.multiple_of(c * XW, XW)
        g = jax.nn.sigmoid(_nn(g8, xT_s[:, pl.ds(c0, XW)])[0:1, :])
        g_s[0, :, pl.ds(c0, XW)] = jnp.broadcast_to(g, (8, XW))
        g_s[1, :, pl.ds(c0, XW)] = jnp.broadcast_to(1.0 - g, (8, XW))
        for t in range(NSLAB):
            proj(t, c0, XW)

    def loop_a(c, carry):
        @pl.when(c == 0)
        def _():
            cp_wB.start()
            cp_woA.start()
            cp_woB.start()
        chunk_a(c)
        return carry

    jax.lax.fori_loop(0, XC - 1, loop_a, 0)
    cp_wB.wait()
    cp_woA.wait()
    cp_woB.wait()
    chunk_a(XC - 1)
    prep_qkv(1)
    woT_s[...] = wo_s[...].astype(F32).T.astype(BF16)

    def loop_b(t, carry):
        proj(t, 0, S)
        return carry

    jax.lax.fori_loop(NSLAB, 2 * NSLAB, loop_b, 0)

    def pair(n1, sw, n2, sr, m2):
        do1 = n1 is not None
        do2 = n2 is not None
        if do1:
            h1 = n1 // NC
            t1 = h1 // 4
            q = q_s[h1, :, pl.ds(pl.multiple_of((n1 % NC) * TQ, TQ), TQ)]
            m8 = jnp.full((8, TQ), -jnp.inf, F32)
        if do2:
            h2 = n2 // NC
            t2 = h2 // 4
            r0 = pl.multiple_of((h2 % 4) * HP, HP)
            c0 = pl.multiple_of((n2 % NC) * TQ, TQ)
            o = jnp.zeros((HP, TQ), F32)

        a = list(range(0, S, KB)) if do1 else []
        bb = list(range(0, S, KB)) if do2 else []
        ia = ib = 0
        while ia < len(a) or ib < len(bb):
            if ia < len(a) and (ib >= len(bb) or a[ia] <= bb[ib] + SKEW * KB):
                k0 = a[ia]
                ia += 1
                s = _nn(k_s[t1, k0:k0 + KB, :], q)
                sw[k0:k0 + KB, :] = s
                m8 = jnp.maximum(m8, jnp.max(s.reshape(KB // 8, 8, TQ), axis=0))
            else:
                k0 = bb[ib]
                ib += 1
                s = sr[k0:k0 + KB, :].reshape(KB // 8, 8, TQ)
                p = jnp.exp2(s - m2[None]).reshape(KB, TQ).astype(BF16)
                o = o + _nn(vT_s[t2, pl.ds(r0, HP), k0:k0 + KB], p)
        if do2:
            sc = g_s[h2 // H, 0:1, pl.ds(c0, TQ)] / o[DH:DH + 1, :]
            oT_s[t2, pl.ds(r0, HP), pl.ds(c0, TQ)] = o * sc
        if do1:
            return jnp.broadcast_to(jnp.max(m8, axis=0, keepdims=True), (8, TQ))
        return None

    def outp(c, carry):
        c0 = pl.multiple_of(c * OC, OC)
        parts = []
        for t in range(2 * NSLAB):
            ot = oT_s[t, :, pl.ds(c0, OC)]
            parts += [ot[HP * i:HP * i + DH] for i in range(4)]
        acc = _nn(woT_s[...], jnp.concatenate(parts, axis=0).astype(BF16))
        out_s[:, pl.ds(c0, OC)] = acc.astype(BF16)
        pltpu.make_async_copy(
            out_s.at[:, pl.ds(c0, OC)], outT_hbm.at[0, :, pl.ds(c0, OC)], out_sem).start()
        return carry

    m0 = pair(0, s0, None, None, None)
    nbody = (NITEM - 2) // (2 * U)

    def body(it, m0):
        for u in range(U):
            n = 2 * (it * U + u)
            m1 = pair(n + 1, s1, n, s0, m0)
            m0 = pair(n + 2, s0, n + 1, s1, m1)
        return m0

    m0 = jax.lax.fori_loop(0, nbody, body, m0)
    for n in range(2 * U * nbody, NITEM - 2, 2):
        m1 = pair(n + 1, s1, n, s0, m0)
        m0 = pair(n + 2, s0, n + 1, s1, m1)
    m1 = pair(NITEM - 1, s1, NITEM - 2, s0, m0)
    pair(None, None, NITEM - 1, s1, m1)

    outp(0, 0)
    jax.lax.fori_loop(1, S // OC, outp, 0)
    pltpu.make_async_copy(out_s, outT_hbm.at[0], out_sem).wait()


@jax.jit
def pallas_gated_mix__mha_block__softmax_full_mha__prompt_kernel(
    A_x: jax.Array,
    A_wqkv: jax.Array,
    A_wo: jax.Array,
    B_x: jax.Array,
    B_wqkv: jax.Array,
    B_wo: jax.Array,
    gate_w: jax.Array,
):
    del B_x
    anyspec = pl.BlockSpec(memory_space=pl.ANY)
    outT = pl.pallas_call(
        _kernel,
        in_specs=[anyspec] * 6,
        out_specs=anyspec,
        out_shape=jax.ShapeDtypeStruct((1, D, S), BF16),
        scratch_shapes=[
            pltpu.VMEM((D, S), BF16),
            pltpu.VMEM((2, D, 3 * D), BF16),
            pltpu.VMEM((2 * D, D), BF16),
            pltpu.VMEM((D,), BF16),
            pltpu.VMEM((D, S), BF16),
            pltpu.VMEM((2 * NSLAB, 3 * SW, D), BF16),
            pltpu.VMEM((D, 2 * D), BF16),
            pltpu.VMEM((2 * NSLAB, S, 128), BF16),
            pltpu.VMEM((2 * H, 128, S), BF16),
            pltpu.VMEM((2 * NSLAB, 128, S), BF16),
            pltpu.VMEM((2 * NSLAB, 128, S), F32),
            pltpu.VMEM((S, TQ), F32),
            pltpu.VMEM((S, TQ), F32),
            pltpu.VMEM((2, 8, S), F32),
            pltpu.SemaphoreType.DMA((8,)),
            pltpu.SemaphoreType.DMA((XC,)),
        ],
        compiler_params=pltpu.CompilerParams(vmem_limit_bytes=110 * 2**20),
    )(jnp.swapaxes(A_x, 1, 2), A_wqkv, A_wo, B_wqkv, B_wo, gate_w)
    return jnp.swapaxes(outT, 1, 2)
```
